```python
import os as _os
_os.environ.setdefault("JAX_PLATFORMS", "cpu")
import jax
import jax.numpy as jnp

def _softmax(x, axis=-1):
    return jax.nn.softmax(x, axis=axis)
def _gelu(x):
    return jax.nn.gelu(x, approximate=True)
def _silu(x):
    return jax.nn.silu(x)
def _sigmoid(x):
    return jax.nn.sigmoid(x)
def _layernorm(x, axis=-1, eps=1e-5):
    m = jnp.mean(x, axis=axis, keepdims=True)
    v = jnp.var(x, axis=axis, keepdims=True)
    return (x - m) / jnp.sqrt(v + eps)
def _scatter_add(tgt, idx, src, axis=0):
    return tgt.at[idx].add(src)
def _segment_sum(src, seg, n):
    return jax.ops.segment_sum(src, seg, n)
class _Rng:
    def __init__(self, key):
        self._k = key
    def _next(self):
        self._k, sub = jax.random.split(self._k)
        return sub
    def normal(self, shape):
        return jax.random.normal(self._next(), shape, dtype=jnp.bfloat16)
    def randint(self, lo, hi, shape):
        return jax.random.randint(self._next(), shape, lo, hi, dtype=jnp.int32)
    def uniform(self, shape, lo=0.0, hi=1.0):
        return jax.random.uniform(self._next(), shape, jnp.bfloat16, lo, hi)
    def permutation(self, n):
        return jax.random.permutation(self._next(), n)


kernel_name = 'sequential_preLN__linear_attn_block__dense_activation_squared_relu__prompt'

def setup_inputs():
    _rng = _Rng(jax.random.key(int.from_bytes(__import__("os").urandom(4), "little")))
    _w = (lambda a: (lambda t: t.astype(jnp.bfloat16) if jnp.issubdtype(t.dtype, jnp.floating) else t)(jnp.asarray(a)))
    def _A_setup():
        B, S, D = 1, 2048, 576
        return {
            "x": _w((lambda *s: _rng.normal(s) * 0.05)(B, S, D)),
            "wqkv": _w((lambda *s: _rng.normal(s) * 0.1)(D, 3 * D)),
            "wo": _w((lambda *s: _rng.normal(s) * 0.05)(D, D)),
        }
    _A_in = _A_setup()

    def _B_setup():
        B, S, D, F = 1, 2048, 576, 4608
        return {
            "x": _w((lambda *s: _rng.normal(s) * 0.05)(B, S, D)),
            "w1": _w((lambda *s: _rng.normal(s) * 0.05)(D, F)),
            "b1": _w((lambda *s: _rng.normal(s) * 0.05)(F)),
            "w2": _w((lambda *s: _rng.normal(s) * 0.05)(F, D)),
            "b2": _w((lambda *s: _rng.normal(s) * 0.05)(D)),
        }
    _B_in = _B_setup()

    return {
        "A_x": _A_in["x"],
        "A_wqkv": _A_in["wqkv"],
        "A_wo": _A_in["wo"],
        "B_x": _B_in["x"],
        "B_w1": _B_in["w1"],
        "B_b1": _B_in["b1"],
        "B_w2": _B_in["w2"],
        "B_b2": _B_in["b2"],
    }

def reference(A_x, A_wqkv, A_wo, B_x, B_w1, B_b1, B_w2, B_b2):
    def _A_ref(x, wqkv, wo):
        B, S, D = x.shape
        H = 32; Dh = D // H
        qkv = (lambda x, *d: x.transpose(*d))((x @ wqkv).reshape(B, S, 3, H, Dh), 2, 0, 3, 1, 4)
        q, k, v = qkv[0], qkv[1], qkv[2]
        phi = lambda t: jnp.where(t > 0, t + 1, jnp.exp(t)) + 1e-6
        pq, pk = phi(q), phi(k)
        kv = jnp.einsum("bhsd,bhse->bhde", pk, v)
        z = jnp.einsum("bhsd->bhd", pk)
        num = jnp.einsum("bhqd,bhde->bhqe", pq, kv)
        den = jnp.einsum("bhqd,bhd->bhq", pq, z)[..., None] + 1e-6
        o = num / den
        return (lambda x, *d: x.transpose(*d))(o, 0, 2, 1, 3).reshape(B, S, D) @ wo

    def _B_ref(x, w1, b1, w2, b2):
        h = jnp.einsum("bsd,df->bsf", x, w1) + b1
        zero = jnp.zeros_like(h)
        r = jnp.where(h > zero, h, zero)
        h = r * r
        out = jnp.einsum("bsf,fd->bsd", h, w2) + b2
        return out

    x = A_x
    h = x + _A_ref(_layernorm(x, axis=-1), A_wqkv, A_wo)
    h2 = h + _B_ref(_layernorm(h, axis=-1), B_w1, B_b1, B_w2, B_b2)
    return h2
```

```python
import functools
import numpy as np
import jax
import jax.numpy as jnp
from jax import lax
import jax.experimental.pallas as pl
import jax.experimental.pallas.tpu as pltpu

S, D, F, H = 2048, 576, 4608, 32
DH = D // H
DP = 640
TM1 = 256
TM2 = 256
FC = 1536
ORDER = "A0B1C2"
bf16 = jnp.bfloat16
f32 = jnp.float32
NT = (((1,), (1,)), ((), ()))


def _dot(a, b):
    return jnp.dot(a, b, preferred_element_type=f32)


def _dot_nt(a, b):
    return lax.dot_general(a, b, NT, preferred_element_type=f32)


def _ln_t(x):
    m = jnp.sum(x, axis=0, keepdims=True) * (1.0 / D)
    xc = x - m
    v = jnp.sum(xc * xc, axis=0, keepdims=True) * (1.0 / D)
    return xc * lax.rsqrt(v + 1e-5)


def _phi(t):
    return jnp.where(t > 0, t + 1.0, jnp.exp(t)) + 1e-6


def _pad_rows(tm, one):
    if not one:
        return jnp.zeros((DP - D, tm), bf16)
    r = lax.broadcasted_iota(jnp.int32, (DP - D, tm), 0)
    return jnp.where(r == 0, 1.0, 0.0).astype(bf16)


def _head(i):
    return (i * 3641) >> 16


def _expand_heads(r):
    tm = r.shape[1]
    row = lax.broadcasted_iota(jnp.int32, (8, tm), 0)
    b = [jnp.broadcast_to(r[h:h + 1, :], (8, tm)) for h in range(H)]
    pieces = []
    for v in range(D // 8):
        h0 = (8 * v) // DH
        h1 = (8 * v + 7) // DH
        if h0 == h1:
            pieces.append(b[h0])
        else:
            pieces.append(jnp.where(row < (DH * h1 - 8 * v), b[h0], b[h1]))
    return jnp.concatenate(pieces, axis=0)


def _band(m):
    lo = 128 * m
    hi = min(D, lo + 128)
    r0 = (lo // DH) * DH
    r1 = -(-hi // DH) * DH
    return (r0 // 16) * 16, -(-r1 // 16) * 16


def kernel(xt_hbm, wqkv_hbm, wo_hbm, w1_hbm, b1_ref, w2t_hbm, b2_ref, out_hbm,
           xt_v, wqkv_v, wo_v, wqkt_v, w1_v, w2t_v, xn_v, pqt_v, g_v, wkvot_v, zt_v, b2t_v, ln2_v, h_v, out_v, sems):
    n1 = S // TM1
    n2 = S // TM2

    def x_cp(i):
        return pltpu.make_async_copy(xt_hbm.at[:, pl.ds(i * TM1, TM1)], xt_v.at[:, pl.ds(i * TM1, TM1)], sems.at[i])

    def o_cp(i):
        t0 = i * TM2 if isinstance(i, int) else pl.multiple_of(i * TM2, TM2)
        return pltpu.make_async_copy(out_v.at[:, pl.ds(t0, TM2)], out_hbm.at[:, pl.ds(t0, TM2)], sems.at[n1 + 4 + i])

    cp_wqkv = pltpu.make_async_copy(wqkv_hbm, wqkv_v.at[pl.ds(0, D)], sems.at[n1])
    cp_wo = pltpu.make_async_copy(wo_hbm, wo_v, sems.at[n1 + 1])
    cp_w1 = pltpu.make_async_copy(w1_hbm, w1_v.at[pl.ds(0, D)], sems.at[n1 + 2])
    cp_w2 = pltpu.make_async_copy(w2t_hbm, w2t_v, sems.at[n1 + 3])
    cp_wqkv.start()
    for i in range(n1):
        x_cp(i).start()
    cp_wo.start()
    cp_w1.start()
    cp_w2.start()

    g_v[...] = jnp.zeros_like(g_v)
    wqkv_v[pl.ds(D, DP - D), :] = jnp.zeros((DP - D, 3 * D), bf16)
    r = lax.broadcasted_iota(jnp.int32, (DP - D, F), 0)
    w1_v[pl.ds(D, DP - D), :] = jnp.where(r == 0, b1_ref[...][None, :].astype(f32), 0.0).astype(bf16)
    b2b = jnp.broadcast_to(b2_ref[...][None, :].astype(f32), (128, D))
    b2t_v[...] = b2b.T

    def ln1(t0):
        x = xt_v[:, pl.ds(t0, TM1)].astype(f32)
        xn_v[:, pl.ds(t0, TM1)] = jnp.concatenate([_ln_t(x).astype(bf16), _pad_rows(TM1, True)], axis=0)

    def proj_kg(t0):
        xn = xn_v[:, pl.ds(t0, TM1)]
        k = _dot(wqkt_v[pl.ds(D, D), :], xn)
        pk = _phi(k).astype(bf16)
        g_v[...] += _dot_nt(pk, xn)

    def proj_q(t0):
        xn = xn_v[:, pl.ds(t0, TM1)]
        q = _dot(wqkt_v[pl.ds(0, D), :], xn)
        pqt_v[:, pl.ds(t0, TM1)] = _phi(q).astype(bf16)

    x_cp(0).wait()
    ln1(0)
    cp_wqkv.wait()
    wqkt_v[...] = wqkv_v[:, 0:2 * D].T

    def p1(i, _):
        t0 = pl.multiple_of(i * TM1, TM1)
        t1 = pl.multiple_of((i + 1) * TM1, TM1)
        pltpu.make_async_copy(xt_hbm.at[:, pl.ds(0, TM1)], xt_v.at[:, pl.ds(0, TM1)], sems.at[i + 1]).wait()
        proj_q(t0)
        proj_kg(t0)
        ln1(t1)
        return _

    lax.fori_loop(0, n1 - 1, p1, 0)

    cp_wo.wait()
    proj_kg((n1 - 1) * TM1)
    proj_q((n1 - 1) * TM1)

    gb = g_v[...].astype(bf16)
    pieces = []
    for m in range(5):
        r0, r1 = _band(m)
        c0, c1 = 128 * m, min(D, 128 * m + 128)
        kv = _dot(gb[r0:r1, :], wqkv_v[:, 2 * D + c0:2 * D + c1])
        hr = _head(lax.broadcasted_iota(jnp.int32, kv.shape, 0) + r0)
        hc = _head(lax.broadcasted_iota(jnp.int32, kv.shape, 1) + c0)
        kvm = jnp.where(hr == hc, kv, 0.0).astype(bf16)
        pieces.append((r0, r1, _dot(kvm, wo_v[c0:c1, :])))
    cuts = sorted({p[0] for p in pieces} | {p[1] for p in pieces})
    segs = []
    for a, b in zip(cuts[:-1], cuts[1:]):
        acc = None
        for (r0, r1, val) in pieces:
            if r0 <= a and b <= r1:
                t = val[a - r0:b - r0, :]
                acc = t if acc is None else acc + t
        segs.append(acc)
    wkvo = jnp.concatenate(segs + [jnp.zeros((DP - D, D), f32)], axis=0).astype(bf16)
    wkvot_v[...] = wkvo.T
    oh = (lax.broadcasted_iota(jnp.int32, (16, 128), 0) == 0) & (lax.broadcasted_iota(jnp.int32, (16, 128), 1) == D - 512)
    z = _dot_nt(jnp.where(oh, 1.0, 0.0).astype(bf16), gb[:, 512:DP])[0:1, :]
    hr2 = lax.broadcasted_iota(jnp.int32, (H, D), 0)
    hc2 = _head(lax.broadcasted_iota(jnp.int32, (H, D), 1))
    zt_v[...] = jnp.where(hr2 == hc2, jnp.broadcast_to(z, (H, D)), 0.0).astype(bf16)

    def prep_a(i):
        t0 = i * TM2 if isinstance(i, int) else pl.multiple_of(i * TM2, TM2)
        pq = pqt_v[:, pl.ds(t0, TM2)]
        den = _dot(zt_v[...], pq)
        rden = 1.0 / (den + 1e-6)
        pqn = (pq.astype(f32) * _expand_heads(rden)).astype(bf16)
        return jnp.concatenate([pqn, _pad_rows(TM2, False)], axis=0)

    def prep_b(i, pqn):
        t0 = i * TM2 if isinstance(i, int) else pl.multiple_of(i * TM2, TM2)
        return xt_v[:, pl.ds(t0, TM2)].astype(f32) + _dot(wkvot_v[...], pqn)

    def prep_c(i, h):
        t0 = i * TM2 if isinstance(i, int) else pl.multiple_of(i * TM2, TM2)
        ln2t = jnp.concatenate([_ln_t(h).astype(bf16), _pad_rows(TM2, True)], axis=0)
        ln2_v[pl.ds(t0, TM2), :] = ln2t.T
        h_v[:, pl.ds(t0, TM2)] = h + jnp.concatenate([b2t_v[...]] * (TM2 // 128), axis=1)

    def ffn_chunk(c, ln2, acc):
        h1 = _dot(ln2, w1_v[:, c * FC:(c + 1) * FC])
        rl = jnp.maximum(h1, 0.0)
        return acc + _dot_nt(w2t_v[:, c * FC:(c + 1) * FC], (rl * rl).astype(bf16))

    prep_c(0, prep_b(0, prep_a(0)))
    cp_w1.wait()
    cp_w2.wait()

    def body(i, with_prep):
        t0 = i * TM2 if isinstance(i, int) else pl.multiple_of(i * TM2, TM2)
        ln2 = ln2_v[pl.ds(t0, TM2), :]
        acc = h_v[:, pl.ds(t0, TM2)]
        pqn = hh = None
        for ch in ORDER:
            if ch.isdigit():
                if int(ch) < F // FC:
                    acc = ffn_chunk(int(ch), ln2, acc)
            elif with_prep:
                if ch == "A":
                    pqn = prep_a(i + 1)
                elif ch == "B":
                    hh = prep_b(i + 1, pqn)
                elif ch == "C":
                    prep_c(i + 1, hh)
        out_v[:, pl.ds(t0, TM2)] = acc.astype(bf16)
        o_cp(i).start()

    def p2(i, _):
        body(i, True)
        return _

    lax.fori_loop(0, n2 - 1, p2, 0)
    body(n2 - 1, False)
    for i in range(n2):
        o_cp(i).wait()


@jax.jit
def pallas_sequential_preLN__linear_attn_block__dense_activation_squared_relu__prompt_kernel(
        A_x, A_wqkv, A_wo, B_x, B_w1, B_b1, B_w2, B_b2):
    xt = A_x.reshape(S, D).T
    hb = pl.BlockSpec(memory_space=pltpu.HBM)
    vm = pl.BlockSpec(memory_space=pltpu.VMEM)
    V = pltpu.VMEM
    out = pl.pallas_call(
        kernel,
        out_shape=jax.ShapeDtypeStruct((D, S), bf16),
        in_specs=[hb, hb, hb, hb, vm, hb, vm],
        out_specs=hb,
        scratch_shapes=[
            V((D, S), bf16), V((DP, 3 * D), bf16), V((D, D), bf16),
            V((2 * D, DP), bf16),
            V((DP, F), bf16), V((D, F), bf16), V((DP, S), bf16), V((D, S), bf16),
            V((D, DP), f32), V((D, DP), bf16), V((H, D), bf16), V((D, 128), f32),
            V((S, DP), bf16), V((D, S), f32),
            V((D, S), bf16),
            pltpu.SemaphoreType.DMA((S // TM1 + 4 + S // TM2,)),
        ],
        compiler_params=pltpu.CompilerParams(vmem_limit_bytes=100 * 2**20),
    )(xt, A_wqkv, A_wo, B_w1, B_b1, B_w2.T, B_b2)
    return out.T.reshape(1, S, D)
```

```python
import jax
import jax.numpy as jnp
from jax import lax
import jax.experimental.pallas as pl
import jax.experimental.pallas.tpu as pltpu

S, D, F, H = 2048, 576, 4608, 32
DH = D // H
DP = 640
TM = 256
NB = S // TM
CH = (0, 1536, 3072, 4608)
QSPLIT = 224
WK_EDGES = (512, 768, 1152)
TAIL_EDGES = (0, 288, 576)
bf16 = jnp.bfloat16
f32 = jnp.float32


def _dot(a, b):
    return jnp.dot(a, b, preferred_element_type=f32)


def _dot_nt(a, b):
    return lax.dot_general(a, b, (((1,), (1,)), ((), ())), preferred_element_type=f32)


def _layernorm_t(x):
    m = jnp.sum(x, axis=0, keepdims=True) * (1.0 / D)
    xc = x - m
    v = jnp.sum(xc * xc, axis=0, keepdims=True) * (1.0 / D)
    return xc * lax.rsqrt(v + 1e-5)


def _phi(t):
    return jnp.where(t > 0, t + 1.0, jnp.exp(t)) + 1e-6


def _pad_rows(one):
    if not one:
        return jnp.zeros((DP - D, TM), bf16)
    r = lax.broadcasted_iota(jnp.int32, (DP - D, TM), 0)
    return jnp.where(r == 0, 1.0, 0.0).astype(bf16)


def _head(i):
    return (i * 3641) >> 16


def _expand_heads(r):
    row = lax.broadcasted_iota(jnp.int32, (8, TM), 0)
    b = [jnp.broadcast_to(r[h:h + 1, :], (8, TM)) for h in range(H)]
    pieces = []
    for v in range(D // 8):
        h0, h1 = (8 * v) // DH, (8 * v + 7) // DH
        pieces.append(b[h0] if h0 == h1 else jnp.where(row < (DH * h1 - 8 * v), b[h0], b[h1]))
    return jnp.concatenate(pieces, axis=0)


def _band(m):
    lo, hi = 128 * m, min(D, 128 * m + 128)
    r0, r1 = (lo // DH) * DH, -(-hi // DH) * DH
    return (r0 // 16) * 16, -(-r1 // 16) * 16


def _kernel(xt_hbm, wqkv_hbm, wo_hbm, w1_hbm, b1_hbm, w2t_hbm, b2_hbm, out_hbm,
            xt_v, wqkv_v, wo_v, wqkt_v, w1_v, w2t_v, b1_v, b2_v, xn_v, pqt_v, g_v, wkvot_v,
            zt_v, b2t_v, ln2_v, h_v, out_v, sem, sem_x, sem_b):
    S_X0, S_X1Q, S_M, S_W, S_O, S_K = 0, 1, 2, 3, 4, 5

    def col0(i):
        return i * TM if isinstance(i, int) else pl.multiple_of(i * TM, TM)

    def x_cp(i, s):
        sl = (slice(None), pl.ds(col0(i), TM))
        return pltpu.make_async_copy(xt_hbm.at[sl], xt_v.at[sl], s)

    def o_cp(i, r0=0, r1=D):
        sl = (pl.ds(r0, r1 - r0), pl.ds(col0(i), TM))
        return pltpu.make_async_copy(out_v.at[sl], out_hbm.at[sl], sem.at[S_O])

    def wqkv_cp(c0, c1, s):
        return pltpu.make_async_copy(wqkv_hbm.at[:, pl.ds(c0, c1 - c0)],
                                     wqkv_v.at[pl.ds(0, D), pl.ds(c0, c1 - c0)], sem.at[s])

    wk_win = list(zip(WK_EDGES[:-1], WK_EDGES[1:]))
    tail = list(zip(TAIL_EDGES[:-1], TAIL_EDGES[1:]))
    cp_x0 = x_cp(0, sem.at[S_X0])
    cp_wk = [wqkv_cp(a, b, S_K + n) for n, (a, b) in enumerate(wk_win)]
    grp_x1q = [x_cp(1, sem.at[S_X1Q]), wqkv_cp(0, 512, S_X1Q)]
    grp_m = [pltpu.make_async_copy(b1_hbm, b1_v, sem.at[S_M]),
             pltpu.make_async_copy(b2_hbm, b2_v, sem.at[S_M]),
             wqkv_cp(2 * D, 3 * D, S_M),
             pltpu.make_async_copy(wo_hbm, wo_v, sem.at[S_M])]
    grp_w = [pltpu.make_async_copy(w1_hbm, w1_v.at[pl.ds(0, D)], sem.at[S_W]),
             pltpu.make_async_copy(w2t_hbm, w2t_v, sem.at[S_W])]

    cp_x0.start()
    for c in cp_wk:
        pl.semaphore_signal(sem_b, 1)
        pl.semaphore_wait(sem_b, 1)
        c.start()
    wqkv_v[pl.ds(D, DP - D), :] = jnp.zeros((DP - D, 3 * D), bf16)

    def ln1(t0):
        x = xt_v[:, pl.ds(t0, TM)].astype(f32)
        xn = jnp.concatenate([_layernorm_t(x).astype(bf16), _pad_rows(True)], axis=0)
        xn_v[:, pl.ds(t0, TM)] = xn
        return xn

    def proj_k(t0):
        return _phi(_dot(wqkt_v[pl.ds(D, D), :], xn_v[:, pl.ds(t0, TM)])).astype(bf16)

    def acc_g(t0, pk):
        g_v[...] += _dot_nt(pk, xn_v[:, pl.ds(t0, TM)])

    def proj_q(t0, r0=0, r1=D):
        q = _dot(wqkt_v[pl.ds(r0, r1 - r0), :], xn_v[:, pl.ds(t0, TM)])
        pqt_v[pl.ds(r0, r1 - r0), pl.ds(t0, TM)] = _phi(q).astype(bf16)

    cp_x0.wait()
    for c in grp_x1q:
        c.start()
    xn0 = ln1(0)
    pks = []
    for n, (a, b) in enumerate(wk_win):
        cp_wk[n].wait()
        if n == len(wk_win) - 1:
            for i in range(2, NB):
                x_cp(i, sem_x.at[i - 2]).start()
        wkt = wqkv_v[:, pl.ds(a, b - a)].T
        wqkt_v[pl.ds(a, b - a), :] = wkt
        pks.append(_phi(_dot(wkt[64:, :] if n == 0 else wkt, xn0)).astype(bf16))
    pk0 = jnp.concatenate(pks, axis=0)
    for c in grp_x1q:
        c.wait()
    for c in grp_m + grp_w:
        c.start()
    g_v[...] = _dot_nt(pk0, xn0)
    wqkt_v[pl.ds(0, 512), :] = wqkv_v[:, pl.ds(0, 512)].T
    proj_q(0)
    ln1(TM)

    def phase1(i, carry):
        t0, t1 = col0(i), col0(i + 1)
        x_cp(i + 1, sem_x.at[i - 1]).wait()
        pk = proj_k(t0)
        proj_q(t0, 0, QSPLIT)
        acc_g(t0, pk)
        proj_q(t0, QSPLIT, D)
        ln1(t1)
        return carry

    lax.fori_loop(1, NB - 1, phase1, 0)

    for c in grp_m:
        c.wait()
    r = lax.broadcasted_iota(jnp.int32, (DP - D, F), 0)
    w1_v[pl.ds(D, DP - D), :] = jnp.where(r == 0, b1_v[...][None, :].astype(f32), 0.0).astype(bf16)
    b2t_v[...] = jnp.broadcast_to(b2_v[...][None, :].astype(f32), (128, D)).T

    def prep_a(i):
        pq = pqt_v[:, pl.ds(col0(i), TM)]
        rden = 1.0 / (_dot(zt_v[...], pq) + 1e-6)
        pqn = (pq.astype(f32) * _expand_heads(rden)).astype(bf16)
        return jnp.concatenate([pqn, _pad_rows(False)], axis=0)

    def prep_b(i, pqn):
        return xt_v[:, pl.ds(col0(i), TM)].astype(f32) + _dot(wkvot_v[...], pqn)

    def prep_c(i, h):
        ln2t = jnp.concatenate([_layernorm_t(h).astype(bf16), _pad_rows(True)], axis=0)
        ln2_v[pl.ds(col0(i), TM), :] = ln2t.T
        h_v[:, pl.ds(col0(i), TM)] = h + jnp.concatenate([b2t_v[...]] * (TM // 128), axis=1)

    def ffn_chunk(c, t0, acc):
        h1 = _dot(ln2_v[pl.ds(t0, TM), :], w1_v[:, CH[c]:CH[c + 1]])
        rl = jnp.maximum(h1, 0.0)
        y = _dot_nt(w2t_v[:, CH[c]:CH[c + 1]], (rl * rl).astype(bf16))
        return y if acc is None else acc + y

    tl = (NB - 1) * TM
    pk = proj_k(tl)
    acc_g(tl, pk)

    gb = g_v[...].astype(bf16)
    oh = ((lax.broadcasted_iota(jnp.int32, (16, 128), 0) == 0)
          & (lax.broadcasted_iota(jnp.int32, (16, 128), 1) == D - 512))
    z = _dot_nt(jnp.where(oh, 1.0, 0.0).astype(bf16), gb[:, 512:DP])[0:1, :]
    hr = lax.broadcasted_iota(jnp.int32, (H, D), 0)
    hc = _head(lax.broadcasted_iota(jnp.int32, (H, D), 1))
    zt_v[...] = jnp.where(hr == hc, jnp.broadcast_to(z, (H, D)), 0.0).astype(bf16)
    kvs = []
    for m in range(5):
        r0, r1 = _band(m)
        c0, c1 = 128 * m, min(D, 128 * m + 128)
        kv = _dot(gb[r0:r1, :], wqkv_v[:, 2 * D + c0:2 * D + c1])
        hr = _head(lax.broadcasted_iota(jnp.int32, kv.shape, 0) + r0)
        hc = _head(lax.broadcasted_iota(jnp.int32, kv.shape, 1) + c0)
        kvs.append(jnp.where(hr == hc, kv, 0.0).astype(bf16))

    pqn = prep_a(0)

    pieces = []
    for m in range(5):
        r0, r1 = _band(m)
        c0, c1 = 128 * m, min(D, 128 * m + 128)
        pieces.append((r0, r1, _dot(kvs[m], wo_v[c0:c1, :])))
    cuts = sorted({p[0] for p in pieces} | {p[1] for p in pieces})
    segs = []
    for a, b in zip(cuts[:-1], cuts[1:]):
        acc = None
        for r0, r1, val in pieces:
            if r0 <= a and b <= r1:
                t = val[a - r0:b - r0, :]
                acc = t if acc is None else acc + t
        segs.append(acc)
    wkvo = jnp.concatenate(segs + [jnp.zeros((DP - D, D), f32)], axis=0).astype(bf16)
    wkvot_v[...] = wkvo.T

    proj_q(tl, 0, QSPLIT)
    h0 = prep_b(0, pqn)
    proj_q(tl, QSPLIT, D)
    prep_c(0, h0)
    for c in grp_w:
        c.wait()

    def block(i, last):
        t0 = col0(i)
        acc = ffn_chunk(0, t0, None)
        if not last:
            pqn = prep_a(i + 1)
        acc = ffn_chunk(1, t0, acc)
        if not last:
            h = prep_b(i + 1, pqn)
        acc = ffn_chunk(2, t0, acc)
        if not last:
            prep_c(i + 1, h)
        res = (acc + h_v[:, pl.ds(t0, TM)]).astype(bf16)
        for a, b in (tail if last else [(0, D)]):
            out_v[pl.ds(a, b - a), pl.ds(t0, TM)] = res[a:b, :]
            o_cp(i, a, b).start()

    def phase2(i, carry):
        block(i, False)
        return carry

    lax.fori_loop(0, NB - 1, phase2, 0)
    block(NB - 1, True)
    for i in range(NB - 1):
        o_cp(i).wait()
    for a, b in tail:
        o_cp(NB - 1, a, b).wait()


@jax.jit
def pallas_sequential_preLN__linear_attn_block__dense_activation_squared_relu__prompt_kernel(
    A_x: jax.Array,
    A_wqkv: jax.Array,
    A_wo: jax.Array,
    B_x: jax.Array,
    B_w1: jax.Array,
    B_b1: jax.Array,
    B_w2: jax.Array,
    B_b2: jax.Array,
):
    V = pltpu.VMEM
    out_t = pl.pallas_call(
        _kernel,
        out_shape=jax.ShapeDtypeStruct((D, S), bf16),
        in_specs=[pl.BlockSpec(memory_space=pltpu.HBM)] * 7,
        out_specs=pl.BlockSpec(memory_space=pltpu.HBM),
        scratch_shapes=[
            V((D, S), bf16),
            V((DP, 3 * D), bf16),
            V((D, D), bf16),
            V((2 * D, DP), bf16),
            V((DP, F), bf16),
            V((D, F), bf16),
            V((F,), bf16),
            V((D,), bf16),
            V((DP, S), bf16),
            V((D, S), bf16),
            V((D, DP), f32),
            V((D, DP), bf16),
            V((H, D), bf16),
            V((D, 128), f32),
            V((S, DP), bf16),
            V((D, S), f32),
            V((D, S), bf16),
            pltpu.SemaphoreType.DMA((7,)),
            pltpu.SemaphoreType.DMA((NB - 2,)),
            pltpu.SemaphoreType.REGULAR,
        ],
        compiler_params=pltpu.CompilerParams(vmem_limit_bytes=100 * 2**20),
    )(A_x.reshape(S, D).T, A_wqkv, A_wo, B_w1, B_b1, B_w2.T, B_b2)
    return out_t.T.reshape(1, S, D)
```

```python
import jax
import jax.numpy as jnp
from jax import lax
import jax.experimental.pallas as pl
import jax.experimental.pallas.tpu as pltpu

S, D, F, H = 2048, 576, 4608, 32
DH = D // H
DP = 640
TM = 256
NB = S // TM
CH = (0, 1536, 3072, 4608)
QSPLIT = 224
WK_EDGES = (512, 768, 1152)
TAIL_EDGES = (0, 288, 576)
bf16 = jnp.bfloat16
f32 = jnp.float32


def _dot(a, b):
    return jnp.dot(a, b, preferred_element_type=f32)


def _dot_nt(a, b):
    return lax.dot_general(a, b, (((1,), (1,)), ((), ())), preferred_element_type=f32)


def _layernorm_t(x):
    m = jnp.sum(x, axis=0, keepdims=True) * (1.0 / D)
    xc = x - m
    v = jnp.sum(xc * xc, axis=0, keepdims=True) * (1.0 / D)
    return xc * lax.rsqrt(v + 1e-5)


def _phi(t):
    return jnp.where(t > 0, t + 1.0, jnp.exp(t)) + 1e-6


def _pad_rows(one):
    if not one:
        return jnp.zeros((DP - D, TM), bf16)
    r = lax.broadcasted_iota(jnp.int32, (DP - D, TM), 0)
    return jnp.where(r == 0, 1.0, 0.0).astype(bf16)


def _head(i):
    return (i * 3641) >> 16


def _expand_heads(r):
    row = lax.broadcasted_iota(jnp.int32, (8, TM), 0)
    b = [jnp.broadcast_to(r[h:h + 1, :], (8, TM)) for h in range(H)]
    pieces = []
    for v in range(D // 8):
        h0, h1 = (8 * v) // DH, (8 * v + 7) // DH
        pieces.append(b[h0] if h0 == h1 else jnp.where(row < (DH * h1 - 8 * v), b[h0], b[h1]))
    return jnp.concatenate(pieces, axis=0)


def _band(m):
    lo, hi = 128 * m, min(D, 128 * m + 128)
    r0, r1 = (lo // DH) * DH, -(-hi // DH) * DH
    return (r0 // 16) * 16, -(-r1 // 16) * 16


def _kernel(xt_hbm, wqkv_hbm, wo_hbm, w1_hbm, b1_hbm, w2t_hbm, b2_hbm, out_hbm,
            xt_v, wqkv_v, wo_v, wqkt_v, w1_v, w2t_v, b1_v, b2_v, xn_v, pqt_v, g_v, wkvot_v,
            zt_v, b2t_v, ln2_v, h_v, out_v, sem, sem_x, sem_b):
    S_X0, S_X1Q, S_M, S_W, S_O, S_K = 0, 1, 2, 3, 4, 5

    def col0(i):
        return i * TM if isinstance(i, int) else pl.multiple_of(i * TM, TM)

    def x_cp(i, s):
        sl = (slice(None), pl.ds(col0(i), TM))
        return pltpu.make_async_copy(xt_hbm.at[sl], xt_v.at[sl], s)

    def o_cp(i, r0=0, r1=D):
        sl = (pl.ds(r0, r1 - r0), pl.ds(col0(i), TM))
        return pltpu.make_async_copy(out_v.at[sl], out_hbm.at[sl], sem.at[S_O])

    def wqkv_cp(c0, c1, s):
        return pltpu.make_async_copy(wqkv_hbm.at[:, pl.ds(c0, c1 - c0)],
                                     wqkv_v.at[pl.ds(0, D), pl.ds(c0, c1 - c0)], sem.at[s])

    wk_win = list(zip(WK_EDGES[:-1], WK_EDGES[1:]))
    tail = list(zip(TAIL_EDGES[:-1], TAIL_EDGES[1:]))
    cp_x0 = x_cp(0, sem.at[S_X0])
    cp_wk = [wqkv_cp(a, b, S_K + n) for n, (a, b) in enumerate(wk_win)]
    grp_x1q = [x_cp(1, sem.at[S_X1Q]), wqkv_cp(0, 512, S_X1Q)]
    grp_m = [pltpu.make_async_copy(b1_hbm, b1_v, sem.at[S_M]),
             pltpu.make_async_copy(b2_hbm, b2_v, sem.at[S_M]),
             wqkv_cp(2 * D, 3 * D, S_M),
             pltpu.make_async_copy(wo_hbm, wo_v, sem.at[S_M])]
    grp_w = [pltpu.make_async_copy(w1_hbm, w1_v.at[pl.ds(0, D)], sem.at[S_W]),
             pltpu.make_async_copy(w2t_hbm, w2t_v, sem.at[S_W])]

    cp_x0.start()
    for c in cp_wk:
        pl.semaphore_signal(sem_b, 1)
        pl.semaphore_wait(sem_b, 1)
        c.start()
    wqkv_v[pl.ds(D, DP - D), :] = jnp.zeros((DP - D, 3 * D), bf16)

    def ln1(t0):
        x = xt_v[:, pl.ds(t0, TM)].astype(f32)
        xn = jnp.concatenate([_layernorm_t(x).astype(bf16), _pad_rows(True)], axis=0)
        xn_v[:, pl.ds(t0, TM)] = xn
        return xn

    def proj_k(t0):
        return _phi(_dot(wqkt_v[pl.ds(D, D), :], xn_v[:, pl.ds(t0, TM)])).astype(bf16)

    def acc_g(t0, pk):
        g_v[...] += _dot_nt(pk, xn_v[:, pl.ds(t0, TM)])

    def proj_q(t0, r0=0, r1=D):
        q = _dot(wqkt_v[pl.ds(r0, r1 - r0), :], xn_v[:, pl.ds(t0, TM)])
        pqt_v[pl.ds(r0, r1 - r0), pl.ds(t0, TM)] = _phi(q).astype(bf16)

    cp_x0.wait()
    for c in grp_x1q:
        c.start()
    xn0 = ln1(0)
    pks = []

    def g_rows(n):
        a, b = max(wk_win[n][0], D) - D, wk_win[n][1] - D
        g_v[pl.ds(a, b - a), :] = _dot_nt(pks[n], xn0)

    for n, (a, b) in enumerate(wk_win):
        cp_wk[n].wait()
        if n == len(wk_win) - 1:
            for i in range(2, NB):
                x_cp(i, sem_x.at[(i - 2) // 3]).start()
        if n > 0:
            g_rows(n - 1)
        wkt = wqkv_v[:, pl.ds(a, b - a)].T
        wqkt_v[pl.ds(a, b - a), :] = wkt
        pks.append(_phi(_dot(wkt[64:, :] if n == 0 else wkt, xn0)).astype(bf16))
    for c in grp_x1q:
        c.wait()
    for c in grp_m + grp_w:
        c.start()
    g_rows(len(wk_win) - 1)
    wqkt_v[pl.ds(0, 512), :] = wqkv_v[:, pl.ds(0, 512)].T
    proj_q(0)
    ln1(TM)

    def phase1(i, carry):
        t0, t1 = col0(i), col0(i + 1)
        pk = proj_k(t0)
        proj_q(t0, 0, QSPLIT)
        acc_g(t0, pk)
        proj_q(t0, QSPLIT, D)
        ln1(t1)
        return carry

    def phase1_group(o, carry):
        for j in range(3):
            x_cp(2 + 3 * o + j, sem_x.at[o]).wait()
        lax.fori_loop(1 + 3 * o, 4 + 3 * o, phase1, 0)
        return carry

    lax.fori_loop(0, (NB - 2) // 3, phase1_group, 0)

    for c in grp_m:
        c.wait()
    r = lax.broadcasted_iota(jnp.int32, (DP - D, F), 0)
    w1_v[pl.ds(D, DP - D), :] = jnp.where(r == 0, b1_v[...][None, :].astype(f32), 0.0).astype(bf16)
    b2t_v[...] = jnp.broadcast_to(b2_v[...][None, :].astype(f32), (128, D)).T

    def prep_a(i):
        pq = pqt_v[:, pl.ds(col0(i), TM)]
        rden = 1.0 / (_dot(zt_v[...], pq) + 1e-6)
        pqn = (pq.astype(f32) * _expand_heads(rden)).astype(bf16)
        return jnp.concatenate([pqn, _pad_rows(False)], axis=0)

    def prep_b(i, pqn):
        return xt_v[:, pl.ds(col0(i), TM)].astype(f32) + _dot(wkvot_v[...], pqn)

    def prep_c(i, h):
        ln2t = jnp.concatenate([_layernorm_t(h).astype(bf16), _pad_rows(True)], axis=0)
        ln2_v[pl.ds(col0(i), TM), :] = ln2t.T
        h_v[:, pl.ds(col0(i), TM)] = h + jnp.concatenate([b2t_v[...]] * (TM // 128), axis=1)

    def ffn_chunk(c, t0, acc):
        h1 = _dot(ln2_v[pl.ds(t0, TM), :], w1_v[:, CH[c]:CH[c + 1]])
        rl = jnp.maximum(h1, 0.0)
        y = _dot_nt(w2t_v[:, CH[c]:CH[c + 1]], (rl * rl).astype(bf16))
        return y if acc is None else acc + y

    tl = (NB - 1) * TM
    pk = proj_k(tl)
    acc_g(tl, pk)

    gb = g_v[...].astype(bf16)
    oh = ((lax.broadcasted_iota(jnp.int32, (16, 128), 0) == 0)
          & (lax.broadcasted_iota(jnp.int32, (16, 128), 1) == D - 512))
    z = _dot_nt(jnp.where(oh, 1.0, 0.0).astype(bf16), gb[:, 512:DP])[0:1, :]
    hr = lax.broadcasted_iota(jnp.int32, (H, D), 0)
    hc = _head(lax.broadcasted_iota(jnp.int32, (H, D), 1))
    zt_v[...] = jnp.where(hr == hc, jnp.broadcast_to(z, (H, D)), 0.0).astype(bf16)
    kvs = []
    for m in range(5):
        r0, r1 = _band(m)
        c0, c1 = 128 * m, min(D, 128 * m + 128)
        kv = _dot(gb[r0:r1, :], wqkv_v[:, 2 * D + c0:2 * D + c1])
        hr = _head(lax.broadcasted_iota(jnp.int32, kv.shape, 0) + r0)
        hc = _head(lax.broadcasted_iota(jnp.int32, kv.shape, 1) + c0)
        kvs.append(jnp.where(hr == hc, kv, 0.0).astype(bf16))

    pqn = prep_a(0)

    pieces = []
    for m in range(5):
        r0, r1 = _band(m)
        c0, c1 = 128 * m, min(D, 128 * m + 128)
        pieces.append((r0, r1, _dot(kvs[m], wo_v[c0:c1, :])))
    cuts = sorted({p[0] for p in pieces} | {p[1] for p in pieces})
    segs = []
    for a, b in zip(cuts[:-1], cuts[1:]):
        acc = None
        for r0, r1, val in pieces:
            if r0 <= a and b <= r1:
                t = val[a - r0:b - r0, :]
                acc = t if acc is None else acc + t
        segs.append(acc)
    wkvo = jnp.concatenate(segs + [jnp.zeros((DP - D, D), f32)], axis=0).astype(bf16)
    wkvot_v[...] = wkvo.T

    proj_q(tl, 0, QSPLIT)
    h0 = prep_b(0, pqn)
    proj_q(tl, QSPLIT, D)
    prep_c(0, h0)
    for c in grp_w:
        c.wait()

    def block(i, last):
        t0 = col0(i)
        acc = ffn_chunk(0, t0, None)
        if not last:
            pqn = prep_a(i + 1)
        acc = ffn_chunk(1, t0, acc)
        if not last:
            h = prep_b(i + 1, pqn)
        acc = ffn_chunk(2, t0, acc)
        if not last:
            prep_c(i + 1, h)
        res = (acc + h_v[:, pl.ds(t0, TM)]).astype(bf16)
        for a, b in (tail if last else [(0, D)]):
            out_v[pl.ds(a, b - a), pl.ds(t0, TM)] = res[a:b, :]
            o_cp(i, a, b).start()

    def phase2(i, carry):
        block(i, False)
        return carry

    lax.fori_loop(0, NB - 1, phase2, 0)
    block(NB - 1, True)
    for i in range(NB - 1):
        o_cp(i).wait()
    for a, b in tail:
        o_cp(NB - 1, a, b).wait()


@jax.jit
def pallas_sequential_preLN__linear_attn_block__dense_activation_squared_relu__prompt_kernel(
    A_x: jax.Array,
    A_wqkv: jax.Array,
    A_wo: jax.Array,
    B_x: jax.Array,
    B_w1: jax.Array,
    B_b1: jax.Array,
    B_w2: jax.Array,
    B_b2: jax.Array,
):
    V = pltpu.VMEM
    out_t = pl.pallas_call(
        _kernel,
        out_shape=jax.ShapeDtypeStruct((D, S), bf16),
        in_specs=[pl.BlockSpec(memory_space=pltpu.HBM)] * 7,
        out_specs=pl.BlockSpec(memory_space=pltpu.HBM),
        scratch_shapes=[
            V((D, S), bf16),
            V((DP, 3 * D), bf16),
            V((D, D), bf16),
            V((2 * D, DP), bf16),
            V((DP, F), bf16),
            V((D, F), bf16),
            V((F,), bf16),
            V((D,), bf16),
            V((DP, S), bf16),
            V((D, S), bf16),
            V((D, DP), f32),
            V((D, DP), bf16),
            V((H, D), bf16),
            V((D, 128), f32),
            V((S, DP), bf16),
            V((D, S), f32),
            V((D, S), bf16),
            pltpu.SemaphoreType.DMA((7,)),
            pltpu.SemaphoreType.DMA(((NB - 2) // 3,)),
            pltpu.SemaphoreType.REGULAR,
        ],
        compiler_params=pltpu.CompilerParams(vmem_limit_bytes=100 * 2**20),
    )(A_x.reshape(S, D).T, A_wqkv, A_wo, B_w1, B_b1, B_w2.T, B_b2)
    return out_t.T.reshape(1, S, D)
```

```python
import jax
import jax.numpy as jnp
from jax import lax
import jax.experimental.pallas as pl
import jax.experimental.pallas.tpu as pltpu

S, D, F, H = 2048, 576, 4608, 32
DH = D // H
DP = 640
TM = 256
NB = S // TM
CH = (0, 1536, 3072, 4608)
QSPLIT = 256
WK_EDGES = (512, 768, 1152)
TAIL_EDGES = (0, 480, 576)
bf16 = jnp.bfloat16
f32 = jnp.float32


def _dot(a, b):
    return jnp.dot(a, b, preferred_element_type=f32)


def _dot_nt(a, b):
    return lax.dot_general(a, b, (((1,), (1,)), ((), ())), preferred_element_type=f32)


def _layernorm_t(x):
    m = jnp.sum(x, axis=0, keepdims=True) * (1.0 / D)
    xc = x - m
    v = jnp.sum(xc * xc, axis=0, keepdims=True) * (1.0 / D)
    return xc * lax.rsqrt(v + 1e-5)


def _phi(t):
    return jnp.where(t > 0, t + 1.0, jnp.exp(t)) + 1e-6


def _pad_rows(one):
    if not one:
        return jnp.zeros((DP - D, TM), bf16)
    r = lax.broadcasted_iota(jnp.int32, (DP - D, TM), 0)
    return jnp.where(r == 0, 1.0, 0.0).astype(bf16)


def _head(i):
    return (i * 3641) >> 16


def _expand_heads(r):
    row = lax.broadcasted_iota(jnp.int32, (8, TM), 0)
    b = [jnp.broadcast_to(r[h:h + 1, :], (8, TM)) for h in range(H)]
    pieces = []
    for v in range(D // 8):
        h0, h1 = (8 * v) // DH, (8 * v + 7) // DH
        pieces.append(b[h0] if h0 == h1 else jnp.where(row < (DH * h1 - 8 * v), b[h0], b[h1]))
    return jnp.concatenate(pieces, axis=0)


def _band(m):
    lo, hi = 128 * m, min(D, 128 * m + 128)
    r0, r1 = (lo // DH) * DH, -(-hi // DH) * DH
    return (r0 // 16) * 16, -(-r1 // 16) * 16


def _kernel(xt_hbm, wqkv_hbm, wo_hbm, w1_hbm, b1_hbm, w2t_hbm, b2_hbm, out_hbm,
            xt_v, wqkv_v, wo_v, wqkt_v, w1_v, w2t_v, b1_v, b2_v, xn_v, pqt_v, g_v, wkvot_v,
            zt_v, b2t_v, ln2_v, h_v, out_v, sem, sem_x, sem_b):
    S_X0, S_X1Q, S_M, S_W, S_O, S_K = 0, 1, 2, 3, 4, 5

    def col0(i):
        return i * TM if isinstance(i, int) else pl.multiple_of(i * TM, TM)

    def x_cp(i, s):
        sl = (slice(None), pl.ds(col0(i), TM))
        return pltpu.make_async_copy(xt_hbm.at[sl], xt_v.at[sl], s)

    def o_cp(i, r0=0, r1=D):
        sl = (pl.ds(r0, r1 - r0), pl.ds(col0(i), TM))
        return pltpu.make_async_copy(out_v.at[sl], out_hbm.at[sl], sem.at[S_O])

    def wqkv_cp(c0, c1, s):
        return pltpu.make_async_copy(wqkv_hbm.at[:, pl.ds(c0, c1 - c0)],
                                     wqkv_v.at[pl.ds(0, D), pl.ds(c0, c1 - c0)], sem.at[s])

    wk_win = list(zip(WK_EDGES[:-1], WK_EDGES[1:]))
    tail = list(zip(TAIL_EDGES[:-1], TAIL_EDGES[1:]))
    cp_x0 = x_cp(0, sem.at[S_X0])
    cp_wk = [wqkv_cp(a, b, S_K + n) for n, (a, b) in enumerate(wk_win)]
    grp_x1q = [x_cp(1, sem.at[S_X1Q]), wqkv_cp(0, 512, S_X1Q)]
    grp_m = [pltpu.make_async_copy(b1_hbm, b1_v, sem.at[S_M]),
             pltpu.make_async_copy(b2_hbm, b2_v, sem.at[S_M]),
             wqkv_cp(2 * D, 3 * D, S_M),
             pltpu.make_async_copy(wo_hbm, wo_v, sem.at[S_M])]
    grp_w = [pltpu.make_async_copy(w1_hbm, w1_v.at[pl.ds(0, D)], sem.at[S_W]),
             pltpu.make_async_copy(w2t_hbm, w2t_v, sem.at[S_W])]

    cp_x0.start()
    for c in cp_wk:
        pl.semaphore_signal(sem_b, 1)
        pl.semaphore_wait(sem_b, 1)
        c.start()
    wqkv_v[pl.ds(D, DP - D), :] = jnp.zeros((DP - D, 3 * D), bf16)

    def ln1(t0):
        x = xt_v[:, pl.ds(t0, TM)].astype(f32)
        xn = jnp.concatenate([_layernorm_t(x).astype(bf16), _pad_rows(True)], axis=0)
        xn_v[:, pl.ds(t0, TM)] = xn
        return xn

    def proj_k(t0):
        return _phi(_dot(wqkt_v[pl.ds(D, D), :], xn_v[:, pl.ds(t0, TM)])).astype(bf16)

    def acc_g(t0, pk):
        g_v[...] += _dot_nt(pk, xn_v[:, pl.ds(t0, TM)])

    def proj_q(t0, r0=0, r1=D):
        q = _dot(wqkt_v[pl.ds(r0, r1 - r0), :], xn_v[:, pl.ds(t0, TM)])
        pqt_v[pl.ds(r0, r1 - r0), pl.ds(t0, TM)] = _phi(q).astype(bf16)

    cp_x0.wait()
    for c in grp_x1q:
        c.start()
    xn0 = ln1(0)
    pks = []

    def g_rows(n):
        a, b = max(wk_win[n][0], D) - D, wk_win[n][1] - D
        g_v[pl.ds(a, b - a), :] = _dot_nt(pks[n], xn0)

    for n, (a, b) in enumerate(wk_win):
        cp_wk[n].wait()
        if n == len(wk_win) - 1:
            for i in range(2, NB):
                x_cp(i, sem_x.at[(i - 2) // 3]).start()
        if n > 0:
            g_rows(n - 1)
        wkt = wqkv_v[:, pl.ds(a, b - a)].T
        wqkt_v[pl.ds(a, b - a), :] = wkt
        pks.append(_phi(_dot(wkt[64:, :] if n == 0 else wkt, xn0)).astype(bf16))
    for c in grp_x1q:
        c.wait()
    for c in grp_m + grp_w:
        c.start()
    g_rows(len(wk_win) - 1)
    wqkt_v[pl.ds(0, 512), :] = wqkv_v[:, pl.ds(0, 512)].T
    proj_q(0)
    ln1(TM)

    def phase1(i, carry):
        t0, t1 = col0(i), col0(i + 1)
        pk = proj_k(t0)
        proj_q(t0, 0, QSPLIT)
        acc_g(t0, pk)
        proj_q(t0, QSPLIT, D)
        ln1(t1)
        return carry

    def phase1_group(o, carry):
        for j in range(3):
            x_cp(2 + 3 * o + j, sem_x.at[o]).wait()
        lax.fori_loop(0, 3, lambda j, c: phase1(1 + 3 * o + j, c), 0)
        return carry

    lax.fori_loop(0, (NB - 2) // 3, phase1_group, 0)

    for c in grp_m:
        c.wait()
    r = lax.broadcasted_iota(jnp.int32, (DP - D, F), 0)
    w1_v[pl.ds(D, DP - D), :] = jnp.where(r == 0, b1_v[...][None, :].astype(f32), 0.0).astype(bf16)
    b2t_v[...] = jnp.broadcast_to(b2_v[...][None, :].astype(f32), (128, D)).T

    def prep_a(i):
        pq = pqt_v[:, pl.ds(col0(i), TM)]
        rden = 1.0 / (_dot(zt_v[...], pq) + 1e-6)
        pqn = (pq.astype(f32) * _expand_heads(rden)).astype(bf16)
        return jnp.concatenate([pqn, _pad_rows(False)], axis=0)

    def prep_b(i, pqn):
        return xt_v[:, pl.ds(col0(i), TM)].astype(f32) + _dot(wkvot_v[...], pqn)

    def prep_c(i, h):
        ln2t = jnp.concatenate([_layernorm_t(h).astype(bf16), _pad_rows(True)], axis=0)
        ln2_v[pl.ds(col0(i), TM), :] = ln2t.T
        h_v[:, pl.ds(col0(i), TM)] = h + jnp.concatenate([b2t_v[...]] * (TM // 128), axis=1)

    def ffn_chunk(c, t0, acc):
        h1 = _dot(ln2_v[pl.ds(t0, TM), :], w1_v[:, CH[c]:CH[c + 1]])
        rl = jnp.maximum(h1, 0.0)
        y = _dot_nt(w2t_v[:, CH[c]:CH[c + 1]], (rl * rl).astype(bf16))
        return y if acc is None else acc + y

    tl = (NB - 1) * TM
    pk = proj_k(tl)
    acc_g(tl, pk)

    gb = g_v[...].astype(bf16)
    oh = ((lax.broadcasted_iota(jnp.int32, (16, 128), 0) == 0)
          & (lax.broadcasted_iota(jnp.int32, (16, 128), 1) == D - 512))
    z = _dot_nt(jnp.where(oh, 1.0, 0.0).astype(bf16), gb[:, 512:DP])[0:1, :]
    hr = lax.broadcasted_iota(jnp.int32, (H, D), 0)
    hc = _head(lax.broadcasted_iota(jnp.int32, (H, D), 1))
    zt_v[...] = jnp.where(hr == hc, jnp.broadcast_to(z, (H, D)), 0.0).astype(bf16)
    kvs = []
    for m in range(5):
        r0, r1 = _band(m)
        c0, c1 = 128 * m, min(D, 128 * m + 128)
        kv = _dot(gb[r0:r1, :], wqkv_v[:, 2 * D + c0:2 * D + c1])
        hr = _head(lax.broadcasted_iota(jnp.int32, kv.shape, 0) + r0)
        hc = _head(lax.broadcasted_iota(jnp.int32, kv.shape, 1) + c0)
        kvs.append(jnp.where(hr == hc, kv, 0.0).astype(bf16))

    pqn = prep_a(0)

    pieces = []
    for m in range(5):
        r0, r1 = _band(m)
        c0, c1 = 128 * m, min(D, 128 * m + 128)
        pieces.append((r0, r1, _dot(kvs[m], wo_v[c0:c1, :])))
    cuts = sorted({p[0] for p in pieces} | {p[1] for p in pieces})
    segs = []
    for a, b in zip(cuts[:-1], cuts[1:]):
        acc = None
        for r0, r1, val in pieces:
            if r0 <= a and b <= r1:
                t = val[a - r0:b - r0, :]
                acc = t if acc is None else acc + t
        segs.append(acc)
    wkvo = jnp.concatenate(segs + [jnp.zeros((DP - D, D), f32)], axis=0).astype(bf16)
    wkvot_v[...] = wkvo.T

    proj_q(tl, 0, QSPLIT)
    h0 = prep_b(0, pqn)
    proj_q(tl, QSPLIT, D)
    prep_c(0, h0)
    for c in grp_w:
        c.wait()

    def block(i, last):
        t0 = col0(i)
        acc = ffn_chunk(0, t0, None)
        if not last:
            pqn = prep_a(i + 1)
        acc = ffn_chunk(1, t0, acc)
        if not last:
            h = prep_b(i + 1, pqn)
        if last:
            rl = jnp.maximum(_dot(ln2_v[pl.ds(t0, TM), :], w1_v[:, CH[2]:CH[3]]), 0.0)
            act = (rl * rl).astype(bf16)
            for a, b in tail:
                rows = pl.ds(a, b - a)
                y = acc[a:b, :] + _dot_nt(w2t_v[rows, CH[2]:CH[3]], act)
                out_v[rows, pl.ds(t0, TM)] = (y + h_v[rows, pl.ds(t0, TM)]).astype(bf16)
                o_cp(i, a, b).start()
            return
        acc = ffn_chunk(2, t0, acc)
        prep_c(i + 1, h)
        out_v[:, pl.ds(t0, TM)] = (acc + h_v[:, pl.ds(t0, TM)]).astype(bf16)
        o_cp(i).start()

    def phase2(i, carry):
        block(i, False)
        return carry

    lax.fori_loop(0, NB - 1, phase2, 0)
    block(NB - 1, True)
    for i in range(NB - 1):
        o_cp(i).wait()
    for a, b in tail:
        o_cp(NB - 1, a, b).wait()


@jax.jit
def pallas_sequential_preLN__linear_attn_block__dense_activation_squared_relu__prompt_kernel(
    A_x: jax.Array,
    A_wqkv: jax.Array,
    A_wo: jax.Array,
    B_x: jax.Array,
    B_w1: jax.Array,
    B_b1: jax.Array,
    B_w2: jax.Array,
    B_b2: jax.Array,
):
    V = pltpu.VMEM
    out_t = pl.pallas_call(
        _kernel,
        out_shape=jax.ShapeDtypeStruct((D, S), bf16),
        in_specs=[pl.BlockSpec(memory_space=pltpu.HBM)] * 7,
        out_specs=pl.BlockSpec(memory_space=pltpu.HBM),
        scratch_shapes=[
            V((D, S), bf16),
            V((DP, 3 * D), bf16),
            V((D, D), bf16),
            V((2 * D, DP), bf16),
            V((DP, F), bf16),
            V((D, F), bf16),
            V((F,), bf16),
            V((D,), bf16),
            V((DP, S), bf16),
            V((D, S), bf16),
            V((D, DP), f32),
            V((D, DP), bf16),
            V((H, D), bf16),
            V((D, 128), f32),
            V((S, DP), bf16),
            V((D, S), f32),
            V((D, S), bf16),
            pltpu.SemaphoreType.DMA((7,)),
            pltpu.SemaphoreType.DMA(((NB - 2) // 3,)),
            pltpu.SemaphoreType.REGULAR,
        ],
        compiler_params=pltpu.CompilerParams(vmem_limit_bytes=100 * 2**20),
    )(A_x.reshape(S, D).T, A_wqkv, A_wo, B_w1, B_b1, B_w2.T, B_b2)
    return out_t.T.reshape(1, S, D)
```
